```python
import os as _os
_os.environ.setdefault("JAX_PLATFORMS", "cpu")
import jax
import jax.numpy as jnp

def _softmax(x, axis=-1):
    return jax.nn.softmax(x, axis=axis)
def _gelu(x):
    return jax.nn.gelu(x, approximate=True)
def _silu(x):
    return jax.nn.silu(x)
def _sigmoid(x):
    return jax.nn.sigmoid(x)
def _layernorm(x, axis=-1, eps=1e-5):
    m = jnp.mean(x, axis=axis, keepdims=True)
    v = jnp.var(x, axis=axis, keepdims=True)
    return (x - m) / jnp.sqrt(v + eps)
def _scatter_add(tgt, idx, src, axis=0):
    return tgt.at[idx].add(src)
def _segment_sum(src, seg, n):
    return jax.ops.segment_sum(src, seg, n)
class _Rng:
    def __init__(self, key):
        self._k = key
    def _next(self):
        self._k, sub = jax.random.split(self._k)
        return sub
    def normal(self, shape):
        return jax.random.normal(self._next(), shape, dtype=jnp.bfloat16)
    def randint(self, lo, hi, shape):
        return jax.random.randint(self._next(), shape, lo, hi, dtype=jnp.int32)
    def uniform(self, shape, lo=0.0, hi=1.0):
        return jax.random.uniform(self._next(), shape, jnp.bfloat16, lo, hi)
    def permutation(self, n):
        return jax.random.permutation(self._next(), n)


kernel_name = 'interleave_layers__sliding_local_dilated__mixer_s_mlp__prompt'

def setup_inputs():
    _rng = _Rng(jax.random.key(int.from_bytes(__import__("os").urandom(4), "little")))
    _w = (lambda a: (lambda t: t.astype(jnp.bfloat16) if jnp.issubdtype(t.dtype, jnp.floating) else t)(jnp.asarray(a)))
    def _A_setup():
        B, S, D = 1, 2048, 448
        return {
            "x": _w((lambda *s: _rng.normal(s) * 0.05)(B, S, D)),
            "wqkv": _w((lambda *s: _rng.normal(s) * 0.05)(D, 3 * D)),
            "wo": _w((lambda *s: _rng.normal(s) * 0.05)(D, D)),
        }
    _A_in = _A_setup()

    def _B_setup():
        B, S, D, F = 1, 2048, 448, 1792
        return {
            "x":  _w((lambda *s: _rng.normal(s) * 0.05)(B, S, D)),
            "w1": _w((lambda *s: _rng.normal(s) * 0.8)(D, D) * (D ** -0.5)),
            "w2": _w((lambda *s: _rng.normal(s) * 0.8)(D, D) * (D ** -0.5)),
            "w3": _w((lambda *s: _rng.normal(s) * 0.8)(D, F) * (D ** -0.5)),
            "w4": _w((lambda *s: _rng.normal(s) * 0.8)(F, D) * (F ** -0.5)),
        }
    _B_in = _B_setup()

    return {
        "A_x": _A_in["x"],
        "A_wqkv": _A_in["wqkv"],
        "A_wo": _A_in["wo"],
        "B_x": _B_in["x"],
        "B_w1": _B_in["w1"],
        "B_w2": _B_in["w2"],
        "B_w3": _B_in["w3"],
        "B_w4": _B_in["w4"],
    }

def reference(A_x, A_wqkv, A_wo, B_x, B_w1, B_w2, B_w3, B_w4):
    def _A_ref(x, wqkv, wo):
        B, S, D = x.shape
        H = 16; Dh = D // H
        W, dil = 8, 2
        qkv = (lambda x, *d: x.transpose(*d))((x @ wqkv).reshape(B, S, 3, H, Dh), 2, 0, 3, 1, 4)
        q, k, v = qkv[0], qkv[1], qkv[2]
        scale = Dh ** -0.5
        pos = jnp.arange(S)
        off = jnp.arange(W) * dil
        idx = pos[:, None] - off[None, :]
        mask = idx >= 0
        idx_c = jnp.where(mask, idx, 0).reshape(-1)
        kg = k[:, :, idx_c, :].reshape(B, H, S, W, Dh)
        vg = v[:, :, idx_c, :].reshape(B, H, S, W, Dh)
        logits = jnp.einsum("bhsd,bhswd->bhsw", q, kg) * scale
        logits = jnp.where(mask[None, None, :, :], logits, -1e9)
        attn = _softmax(logits, axis=-1)
        o = jnp.einsum("bhsw,bhswd->bhsd", attn, vg)
        return (lambda x, *d: x.transpose(*d))(o, 0, 2, 1, 3).reshape(B, S, D) @ wo

    def _B_ref(x, w1, w2, w3, w4):
        B, S, D = x.shape
        h = _gelu(_layernorm(x, axis=-1) @ w1)
        c = D // 4
        g0 = jnp.pad(h[:, :, 0*c:1*c], ((0, 0), (1, 0), (0, 0)))[:, :S, :]
        g1 = jnp.pad(h[:, :, 1*c:2*c], ((0, 0), (0, 1), (0, 0)))[:, 1:, :]
        g2 = jnp.pad(h[:, :, 2*c:3*c], ((0, 0), (2, 0), (0, 0)))[:, :S, :]
        g3 = jnp.pad(h[:, :, 3*c:   ], ((0, 0), (0, 2), (0, 0)))[:, 2:, :]
        hs = jnp.concatenate([g0, g1, g2, g3], axis=-1) @ w2
        x1 = x + hs
        h2 = _gelu(_layernorm(x1, axis=-1) @ w3) @ w4
        return x1 + h2

    x = A_x
    x = x + _A_ref(_layernorm(x, axis=-1), A_wqkv, A_wo)
    x = x + _B_ref(_layernorm(x, axis=-1), B_w1, B_w2, B_w3, B_w4)
    x = x + _A_ref(_layernorm(x, axis=-1), A_wqkv, A_wo)
    x = x + _B_ref(_layernorm(x, axis=-1), B_w1, B_w2, B_w3, B_w4)
    return x
```

```python
import numpy as np
import jax
import jax.numpy as jnp
from jax.experimental import pallas as pl
from jax.experimental.pallas import tpu as pltpu

S, D, H, DH, WIN, DIL, F = 2048, 448, 16, 28, 8, 2, 1792
TT = 128
NP = S // (2 * TT)
K1 = 256
KP = 2 * K1
CG = D // 4
NC3 = 4
RB = 32
EPS = 1e-5
f32, bf16, u32 = jnp.float32, jnp.bfloat16, jnp.uint32

ORD = (1, 3, 2, 4, 0, 5, 6)
GROUPS = "x0.x1.wq wkv.x2 wo.w1.w2.x3.x4.x5 x6.x7.w3.w4"
STARTS = (-1, -1, -1, 1)
ORDER = (
    "DMA.0 Q.0 DMA.1 Q.1 K.0 Q.2 V.0 K.1 V.1 K.2 DMA.2 Q.3 K.3 K.4 Q.4 V.2 WO.0 Q.5 K.5 DMA.3 V.3 V.4 K.6 Q.6 "
    "WO.1 V.5 W1.0 Q.7 V.6 WO.2 V.7 W1.1 K.7 W2.0 WO.3 W1.2 W30.0 W2.1 W31.0 W32.0 W33.0 WO.4 W1.3 W4.0 W2.2 "
    "W30.1 W32.1 W33.1 W31.1 WO.5 W1.4 Q.8 K.8 V.8 W4.1 W2.3 W30.2 W31.2 W33.2 W32.2 WO.6 W1.5 Q.9 K.9 V.9 W4.2 "
    "W2.4 W30.3 W31.3 W32.3 W33.3 WO.7 W1.6 Q.10 K.10 V.10 W4.3 W2.5 W30.4 W31.4 W32.4 W33.4 WO.8 Q.11 W1.7 K.11 "
    "W30.5 V.11 W4.4 W2.6 W31.5 W32.5 W33.5 WO.9 W1.8 Q.12 K.12 V.12 W31.6 W4.5 W2.7 W30.6 W33.6 W32.6 WO.10 W1.9 "
    "K.13 Q.13 V.13 W4.6 W30.7 W2.8 W31.7 W32.7 W33.7 WO.11 W1.10 Q.14 K.14 V.14 W4.7 W2.9 W30.8 W32.8 W31.8 "
    "W33.8 K.15 WO.12 W1.11 V.15 W4.8 W2.10 Q.15 W30.9 W31.9 W32.9 W33.9 WO.13 W1.12 W4.9 W2.11 W30.10 W31.10 "
    "W32.10 W33.10 WO.14 W1.13 W4.10 W2.12 W30.11 W31.11 W32.11 W33.11 WO.15 W1.14 W4.11 W30.12 W2.13 W31.12 "
    "W32.12 W33.12 W1.15 W4.12 W2.14 W30.13 W31.13 W32.13 W33.13 W4.13 W2.15 W30.14 W31.14 W32.14 W33.14 W30.15 "
    "W31.15 W32.15 W33.15 W4.14 W4.15 "
)
PHASES = [
    (0, 1.9, 3.2, 0.36, 0.4, 2, 0, 4, 1),
    (38, 1.9, 3.2, 0.36, 0.4, 2, 0, 4, 1),
    (84, 2.05, 2.7, 0.36, 0.4, 2, 0, 4, 1),
    (133, 1.9, 3.2, 0.36, 0.4, 2, 0, 4, 1),
    (206, 2.05, 2.7, 0.39, 0.32, 3, 1, 4, 1),
    (271, 1.9, 3.2, 0.34, 0.36, 3, 1, 4, 1),
    (344, 1.9, 3.2, 0.34, 0.36, 3, 1, 4, 1),
    (409, 1.9, 3.2, 0.34, 0.41, 3, 0, 99, 1),
    (486, 1.9, 3.2, 0.34, 0.36, 3, 1, 4, 1),
    (563, 1.9, 3.2, 0.28, 0.36, 3, 1, 3, 1),
    (644, 1.9, 3.2, 0.34, 0.36, 3, 1, 7, 1),
]
COST = dict(LA=(812, 0), QK=(3040, 784), PV=(3024, 784), LL=(1288, 0), SH=(224, 224), L1=(700, 0), FO0=(1120, 0), FO1=(1120, 0),
            FO2=(1120, 0), FO3=(1120, 0), cW1=(896, 0), cQ=(336, 0), cK=(336, 0), cV=(336, 0), cWO=(336, 0), cW2=(336, 0),
            cW4=(336, 0), PQ=(1224, 128), PK=(1128, 96), PV_=(1224, 128), PWO=(1560, 128), PW1=(1224, 128), PW2=(1480, 128),
            PW30=(1344, 128), PW31=(1344, 128), PW32=(1344, 128), PW33=(672, 64), PW4=(3528, 0))
GAPS = dict(LA=3, LL=6, L1=3, QK=9, PV=9, SH=2, FO0=1, FO1=1, FO2=1, FO3=1)

GELU_IN = float((0.044715 * np.sqrt(2.0 / np.pi)) ** (1.0 / 3.0))
GELU_OUT = 0.5 / GELU_IN


def _gelu(y):
    return y + y * jnp.tanh(y * (y * y + float(np.sqrt(2.0 / np.pi)) / GELU_IN))


def _cat(parts):
    return parts[0] if len(parts) == 1 else jnp.concatenate(parts, axis=0)


def _weight_operands(w11, w12, w21, w22):
    return [w11 + w22, w21 + w22, w11, w22, w11 + w12, w21 - w11, w12 - w22]


class _Rows:
    def __init__(self):
        self.parts = {}

    def put(self, r0, v):
        self.parts[r0] = v

    def get(self, r0, n):
        out = []
        for k in sorted(self.parts):
            v = self.parts[k]
            lo, hi = max(k, r0), min(k + v.shape[0], r0 + n)
            if lo < hi:
                out.append(v if hi - lo == v.shape[0] else v[lo - k:hi - k])
        assert sum(o.shape[0] for o in out) == n
        return _cat(out)


def _arrival(name):
    return "DMA", [name in g.split(".") for g in GROUPS.split()].index(True)


def _prereqs(key):
    name, i = key
    first, last = i % NP == 0, i % NP == NP - 1
    if name in ("Q", "K", "V"):
        return [("LA", i), ({"Q": "PQ", "K": "PK", "V": "PV_"}[name], 0)]
    if name in ("WO", "W1", "W2", "W4"):
        return [({"WO": "PV", "W1": "LL", "W2": "SH", "W4": "FO3"}[name], i), ("P" + name, 0)]
    if name[:2] == "W3":
        return [("L1", i), ("PW3" + name[2], 0)]
    if name == "LA":
        return [("cW4", i - NP)] if i >= NP else [_arrival("x%d" % i)] + ([("LA", i - 1)] if i else [])
    if name == "QK":
        return [("cQ", i), ("cK", i)] + ([] if first else [("cK", i - 1)])
    if name == "PV":
        return [("QK", i), ("cV", i)] + ([] if first else [("cV", i - 1)])
    if name == "LL":
        return [("cWO", i)]
    if name == "SH":
        return [("cW1", i)] + ([] if first else [("cW1", i - 1)]) + ([] if last else [("cW1", i + 1)])
    if name == "L1":
        return [("cW2", i)]
    if name[:2] == "FO":
        return [("cW3" + name[2], i)] + ([("FO%d" % (int(name[2]) - 1), i)] if name[2] != "0" else [])
    if name == "OUT":
        return [("cW4", i)]
    chain = ["PQ", "PK", "PV_", "PWO", "PW1", "PW2"] + ["PW3%d" % c for c in range(NC3)] + ["PW4"]
    if name not in chain:
        return []
    src = {"PQ": "wq", "PK": "wkv", "PV_": "wkv"}.get(name, name[1:3].lower())
    return [_arrival(src)] + ([(chain[chain.index(name) - 1], 0)] if name != "PQ" else [])


NEXT = (0, 0)


class _Interleaver:
    def __init__(self, order):
        self.deadline, tiles = {}, 0
        starts = []
        for name, _ in order:
            starts.append(tiles / 4)
            tiles += {"W4": 49, "DMA": 0}.get(name, 14)
        for key, start in reversed(list(zip(order, starts))):
            self._mark(key, start)
        self.left = {k: list(COST.get(k[0], (0, 0))) for k in self.deadline}
        self.by_deadline = sorted(self.deadline, key=lambda k: (self.deadline[k], k))
        self.jobs, self.done, self.held, self.due = {}, set(), set(), []
        self.round, self.tiles, self.valu, self.xlu = 0, 0, 0.0, 0.0
        self.delay, _, self.qk_every, self.ln_every = PHASES[0][5:]

    def _mark(self, key, start):
        for k in _prereqs(key):
            self.deadline[k] = start
            self._mark(k, start - GAPS.get(k[0], 0))

    def add(self, key, gen, delay=0):
        self.jobs.setdefault(key, []).append((gen, self.round + delay))

    def hold(self, key):
        self.held.add(key)

    def release(self, key):
        self.held.discard(key)

    def take(self):
        due, self.due = self.due, []
        return due

    def _step(self, key):
        cost = next(self.jobs[key][0][0], None)
        if cost:
            if key in self.left:
                self.left[key] = [max(a - b, 0) for a, b in zip(self.left[key], cost)]
        else:
            self.jobs[key].pop(0)
            if not self.jobs[key]:
                del self.jobs[key]
                if key not in self.held:
                    self.done.add(key)
        return cost

    def need(self, key):
        for k in _prereqs(key):
            if k not in self.done:
                assert k in self.jobs, (key, k)
                self.need(k)
                while k in self.jobs:
                    self._step(k)

    def tick(self, cycles, own):
        self.round += 1
        _, vmin, vmax, xmin, xmax, self.delay, margin, self.qk_every, self.ln_every = [p for p in PHASES if p[0] <= self.round][-1]
        work, rate = [0, 0], [vmin * cycles - own, xmin * cycles]
        for k in self.by_deadline:
            if k not in self.done:
                rounds = max(self.deadline[k] - self.round + 1 - margin, 1)
                work = [a + b for a, b in zip(work, self.left[k])]
                rate = [max(a, b / rounds) for a, b in zip(rate, work)]
        self.valu = min(self.valu, 0.0) + min(rate[0], vmax * cycles - own)
        self.xlu = min(self.xlu, 0.0) + min(rate[1], xmax * cycles)
        skip = set()
        while self.valu > 0:
            ready = [k for k, g in self.jobs.items() if k not in skip and g[0][1] <= self.round
                     and all(p in self.done for p in _prereqs(k))]
            if not ready:
                break
            key = min(ready, key=lambda k: self.deadline.get(k, -1))
            cost = self._step(key)
            if cost is NEXT:
                skip.add(key)
            elif cost:
                self.valu -= cost[0]
                self.xlu -= cost[1]
                self.due.append(cost)
                if cost[1] and self.xlu <= 0:
                    skip.update(k for k in self.jobs if k[0] in ("QK", "PV", "SH") or k[0][0] == "P")


def _kernel(x_hbm, wqkv_hbm, wo_hbm, w1_hbm, w2_hbm, w3_hbm, w4t_hbm, out_hbm,
            xin, wqkv_r, wo_r, w1_r, w2_r, w3_r, w4_r,
            wq_s, wk_s, wv_s, wo_s, w1_s, w2_s, w3_s, w4_s, tmp, pack,
            obuf, sem_x, sem_w, sem_o):
    def xcopy(j):
        return pltpu.make_async_copy(x_hbm.at[:, pl.ds(j * 2 * TT, 2 * TT)], xin.at[j], sem_x.at[j])

    def ocopy(j):
        return pltpu.make_async_copy(obuf.at[j], out_hbm.at[:, pl.ds(j * 2 * TT, 2 * TT)], sem_o.at[j])

    wc = {n: pltpu.make_async_copy(s, d, sem_w.at[i]) for i, (n, s, d) in enumerate(
        [("wq", wqkv_hbm.at[:, pl.ds(0, KP)], wqkv_r.at[pl.ds(0, D), pl.ds(0, KP)]),
         ("wkv", wqkv_hbm.at[:, pl.ds(KP, 3 * D - KP)], wqkv_r.at[pl.ds(0, D), pl.ds(KP, 3 * D - KP)]),
         ("wo", wo_hbm, wo_r.at[pl.ds(0, D)]), ("w1", w1_hbm, w1_r.at[pl.ds(0, D)]), ("w2", w2_hbm, w2_r.at[pl.ds(0, D)]),
         ("w3", w3_hbm, w3_r.at[pl.ds(0, D)]), ("w4", w4t_hbm, w4_r)])}
    lane = jax.lax.broadcasted_iota(jnp.int32, (H, TT), 1)
    order = [(t.split(".")[0], int(t.split(".")[1])) for t in ORDER.split()]
    il = _Interleaver(order)
    val = {}

    def rows(*key):
        return val.setdefault(key, _Rows())

    def put_operands(dst, r0, top, bot):
        nk, n = len(top) // 2, top[0].shape[0]
        out = []
        for c in range(nk):
            for j, o in enumerate(_weight_operands(top[c], top[nk + c], bot[c], bot[nk + c])):
                dst[j, c, r0:r0 + n, :] = o.astype(bf16)
                out.append(dst.bitcast(u32)[j, c, r0 // 2:(r0 + n) // 2, :])
        return out

    def transposed(src, c0, n):
        t = src[:, c0:c0 + n].T
        return [t[:, k:k + 128].astype(f32) for k in range(0, KP, 128)]

    def p_qkv(part):
        dst = (wq_s, wk_s, wv_s)[part]
        for c in range(-(-part * D // 128) * 128, (part + 1) * D, 128):
            n = min(128, 3 * D - c)
            for kt, t in enumerate(transposed(wqkv_r, c, n)):
                tmp[kt, c:c + n, :] = t
            yield 96, 32

        def head_rows(d):
            return [tmp[kt, pl.ds(part * D + d, H, stride=DH), :] for kt in range(KP // 128)]
        for d in range(DH // 2):
            yield (60, 0, *put_operands(dst, d * H, head_rows(d), head_rows(d + DH // 2)))

    def p_square(dst, t):
        for r in range(0, D // 2, 16):
            yield (60, 0, *put_operands(dst, r, [k.get(r, 16) for k in t], [k.get(D // 2 + r, 16) for k in t]))

    def p_wo():
        base = 3 * D
        t = [_Rows() for _ in range(KP // 128)]
        for c in range(0, D, 128):
            n = min(128, D - c)
            a = wo_r[0:D, c:c + n].astype(f32)
            tmp[c // 128, base:base + D, :] = a if n == 128 else jnp.concatenate([a, jnp.zeros((D, 128 - n), f32)], axis=1)
            a = [tmp[c // 128, pl.ds(base + d, H, stride=DH), :][:, 0:n] for d in range(DH)]
            a = _cat(a + [jnp.zeros((KP - D, n), f32)]).astype(bf16).T
            for k in range(KP // 128):
                t[k].put(c, a[:, k * 128:(k + 1) * 128].astype(f32))
            yield 180, 32
        yield from p_square(wo_s, t)

    def p_plain(src, dst, scale):
        t = [_Rows() for _ in range(KP // 128)]
        for c in range(0, D, 128):
            for k, v in enumerate(transposed(src, c, min(128, D - c))):
                t[k].put(c, v if scale == 1 else v * scale)
            yield 96 + 64 * (scale != 1), 32
        yield from p_square(dst, t)

    def p_w3(part):
        n = F // 2 // NC3
        for c in range(-(-part * n // 128) * 128, (part + 1) * n, 128):
            top, bot = transposed(w3_r, c, 128), transposed(w3_r, F // 2 + c, 128)
            yield 192, 64
            for r in range(0, 128, 16):
                yield (60, 0, *put_operands(w3_s, c + r, [t[r:r + 16] for t in top], [t[r:r + 16] for t in bot]))

    def p_w4():
        for r in range(0, D // 2, 16):
            top, bot = [[w4_r[a:a + 16, k:k + 128].astype(f32) for k in range(0, F, 128)] for a in (r, D // 2 + r)]
            yield (252, 0, *put_operands(w4_s, r, top, bot))

    def colsums(get):
        acc = [None, None]
        for r in range(0, D, 64):
            for u in range(2):
                v = jnp.sum(get(u, r).reshape(8, 8, TT), axis=0)
                acc[u] = v if acc[u] is None else acc[u] + v
            yield acc if r // 64 % il.ln_every == il.ln_every - 1 or r == D - 64 else []

    def layernorm(gets, outs, lead, gain=1):
        for acc in colsums(lambda u, r: gets[u](r, 64)):
            yield (16 + lead + len(acc), 0, *acc)
        yield NEXT
        m = [jnp.sum(a, axis=0, keepdims=True) * (1.0 / D) for a in acc]

        def sq(u, r):
            d = gets[u](r, 64) - m[u]
            return d * d
        for acc in colsums(sq):
            yield (48 + len(acc), 0, *acc)
        yield NEXT
        rs = [jax.lax.rsqrt(jnp.sum(a, axis=0, keepdims=True) * (1.0 / D) + EPS) for a in acc]
        rs = rs if gain == 1 else [x * gain for x in rs]
        for r in range(0, D, 64):
            for u in range(2):
                outs[u].put(r, (gets[u](r, 64) - m[u]) * rs[u])

    def operands(name, i, src, k1, k2, lo, hi, cost):
        ops = [rows(name, i, n) for n in range(7)]
        xa, xb = rows(src, i, 0), rows(src, i, 1)
        for r in range(lo, hi, RB):
            x11, x12 = xa.get(r, RB), xb.get(r, RB)
            if r < k2:
                x21, x22 = xa.get(k1 + r, RB), xb.get(k1 + r, RB)
                new = [x11 + x22, x11, x12 - x22, x11 - x21, x22, x11 + x12, x21 + x22]
            else:
                z = jnp.zeros_like(x11)
                new = [x11, x11, x12, x11, z, x11 + x12, z]
            if name == "f_op":
                for n, v in enumerate(new):
                    pack[n, 0:RB, :] = v.astype(bf16)
                    new[n] = pack.bitcast(u32)[n, 0:RB // 2, :]
                    ops[n].put(r // 2, new[n])
                yield ((4 * cost + 8.5) * RB // 8 + 7 * RB // 16, 0, *new)
                continue
            for o, v in zip(ops, new):
                o.put(r, v)
            if name == "o_op":
                continue
            yield ((4 * cost + 4) * RB // 8, 0, new[5], new[6]) if r < k2 else ((2 * cost + 2) * RB // 8, 0, new[5])

    def pad_operands(name, i, src, cost):
        return operands(name, i, src, K1, D - K1, 0, K1, cost)

    def get_x(i, u):
        if i < NP:
            return lambda r, n: xin[i, r:r + n, u * TT:(u + 1) * TT].astype(f32)
        return rows("x", i, u).get

    def shifted(prev, cur, s):
        return cur if s == 0 else pltpu.roll(jnp.where(lane >= TT - s, prev, cur), s, axis=1)

    def g_la(i):
        if i == 0:
            val["never"] = (pltpu.bitcast(xin[0, 0:16, 0:TT], u32) & 1) > 1
        yield from layernorm([get_x(i, u) for u in range(2)], [rows("a", i, u) for u in range(2)], 16 if i < NP else 0)
        yield from pad_operands("a_op", i, "a", 1)

    def g_qk(i):
        for u in range(2):
            acc = [None] * WIN
            first = u == 0 and i % NP == 0
            for d in range(DH):
                q, cur = rows("q", i, u).get(d * H, H), rows("k", i, u).get(d * H, H)
                prev = cur if first else rows("k", i - 1 + u, 1 - u).get(d * H, H)
                for w in range(WIN):
                    x = q * shifted(prev, cur, DIL * w)
                    acc[w] = x if acc[w] is None else acc[w] + x
                yield (62, 14, *acc) if d % il.qk_every == il.qk_every - 1 else (46, 14)
            if u == 1:
                yield NEXT
            lg = acc
            if first:
                lg = [lg[0]] + [jnp.where(lane >= DIL * w, lg[w], -1e9 * DH ** 0.5) for w in range(1, WIN)]
            mx = lg[0]
            for w in range(1, WIN):
                mx = jnp.maximum(mx, lg[w])
            e = [jnp.exp2((x - mx) * (DH ** -0.5 * float(np.log2(np.e)))) for x in lg]
            den = e[0]
            for w in range(1, WIN):
                den = den + e[w]
            inv = 1.0 / den
            val["p", i, u] = [x * inv for x in e]
            yield (120, 0, *val["p", i, u])

    def g_pv(i):
        if i % NP == 0:
            v0 = [jnp.broadcast_to(rows("v", i, 0).get(d * H, H)[:, 0:1], (H, TT)) for d in range(DH)]
            for d in range(0, DH, 4):
                yield (8, 8, *v0[d:d + 4])
            yield NEXT
        for u in range(2):
            p = val["p", i, u]
            for d in range(DH):
                cur = rows("v", i, u).get(d * H, H)
                if u == 0 and i % NP == 0:
                    prev = v0[d]
                else:
                    prev = rows("v", i - 1 + u, 1 - u).get(d * H, H)
                a = None
                for w in range(WIN):
                    x = p[w] * shifted(prev, cur, DIL * w)
                    a = x if a is None else a + x
                rows("o", i, u).put(d * H, a)
                yield 50, 14, a
        yield from pad_operands("o_op", i, "o", 0)

    def g_ll(i):
        yield from layernorm([rows("x1", i, u).get for u in range(2)], [rows("xn", i, u) for u in range(2)], 0)
        yield from layernorm([rows("xn", i, u).get for u in range(2)], [rows("l", i, u) for u in range(2)], 16, GELU_IN)
        yield from pad_operands("l_op", i, "l", 1)

    def g_sh(i):
        for u in range(2):
            for g, s in enumerate((1, -1, 2, -2)):
                for r in range(g * CG, (g + 1) * CG, H):
                    cur = rows("h", i, u).get(r, H)
                    if s > 0:
                        edge = u == 0 and i % NP == 0
                        nb = jnp.zeros_like(cur) if edge else rows("h", i - 1 + u, 1 - u).get(r, H)
                        y = pltpu.roll(jnp.where(lane >= TT - s, nb, cur), s, axis=1)
                    else:
                        edge = u == 1 and i % NP == NP - 1
                        nb = jnp.zeros_like(cur) if edge else rows("h", i + u, 1 - u).get(r, H)
                        y = pltpu.roll(jnp.where(lane < -s, nb, cur), TT + s, axis=1)
                    rows("g", i, u).put(r, y)
        for c in pad_operands("g_op", i, "g", 1):
            yield (c[0], 4 * (len(c) - 2) * RB // 16, *c[2:])

    def g_l1(i):
        yield from layernorm([rows("x2", i, u).get for u in range(2)], [rows("m", i, u) for u in range(2)], 0, GELU_IN)
        yield from pad_operands("m_op", i, "m", 1)

    def g_out(i):
        for r in range(0, D, 64):
            y = jnp.concatenate([rows("x", i + NP, u).get(r, 64) for u in range(2)], axis=1)
            obuf[i - NP, r:r + 64, :] = y.astype(bf16)
            yield 16, 0
        ocopy(i - NP).start()

    def weights(w_ref, j, r0, n, own):
        tiles = []
        for c in range(w_ref.shape[1]):
            if il.tiles % 4 == 0:
                il.tick(n, own)
                leaves = [v if v.dtype == u32 else pltpu.bitcast(v, u32) for item in il.take() for v in item[2:]]
                leaves = [v[r:r + 8] for v in leaves for r in range(0, v.shape[0], 8)]
                val["due"] = [(k / len(leaves), v) for k, v in enumerate(leaves)]
            w = w_ref.bitcast(u32)[j, c, r0 // 2:(r0 + n) // 2, :]
            mine = val["due"][il.tiles % 4::4]
            if mine:
                parts = [w[r:r + 8] for r in range(0, n // 2, 8)]
                for t, v in mine:
                    r = min(int(t * len(parts)), len(parts) - 1)
                    parts[r] = jnp.where(val["never"], v, parts[r])
                w = _cat(parts)
            tiles.append(w)
            il.tiles += 1
        return pltpu.bitcast(jnp.concatenate(tiles, axis=1), bf16)

    def block(name, i):
        il.need((name, i))
        n, r0, k, tied, cost = D // 2, 0, K1, True, 0
        if name[:2] == "W3":
            n = F // 2 // NC3
            r0 = int(name[2]) * n
            w_ref, src, dst, half_rows, f = w3_s, "m_op", "f", F // 2, lambda u, r, v: _gelu(v)
            tied = False
        else:
            half_rows = D // 2
            w_ref, src, dst, f = {
                "Q": (wq_s, "a_op", "q", None), "K": (wk_s, "a_op", "k", None), "V": (wv_s, "a_op", "v", None),
                "WO": (wo_s, "o_op", "x1", lambda u, r, v: get_x(i, u)(r, RB) + v),
                "W1": (w1_s, "l_op", "h", lambda u, r, v: _gelu(v)),
                "W2": (w2_s, "g_op", "x2", lambda u, r, v: rows("xn", i, u).get(r, RB) + v),
                "W4": (w4_s, "f_op", "x", lambda u, r, v: rows("x1", i, u).get(r, RB) + rows("x2", i, u).get(r, RB) + GELU_OUT * v),
            }[name]
            if name == "W4":
                k = F // 2
            if name == "W1":
                tied, cost = True, 5
        m = {}

        def combine(u, half, comb, nadd):
            for r in range(0, n, RB):
                v = comb(lambda j: m[j][r:r + RB])
                ro = half * half_rows + r0 + r
                v = v if f is None else f(u, ro, v)
                rows(dst, i + NP if name == "W4" else i, u).put(ro, v)
                if tied:
                    yield (nadd + cost + 1) * RB // 8, 0, v
        outs = {1: (0, 1, lambda p: p(1) - p(3), 1), 3: (1, 0, lambda p: p(2) + p(4), 1),
                5: (1, 1, lambda p: ((p(2) - p(1)) + p(0)) + p(5), 3), 6: (0, 0, lambda p: (p(0) - (p(3) + p(4))) + p(6), 3)}
        il.hold(("c" + name, i))
        for pos, j in enumerate(ORD):
            x = rows(src, i, j).get(0, k // 2 if src == "f_op" else k)
            x = pltpu.bitcast(x, bf16) if src == "f_op" else x.astype(bf16)
            m[j] = jnp.dot(weights(w_ref, j, r0, n, 200 if name == "W4" else 88), x, preferred_element_type=f32)
            if pos in outs:
                il.add(("c" + name, i), combine(*outs[pos]), delay=il.delay)
        il.release(("c" + name, i))

    groups = [[wc[n] if n[0] == "w" else xcopy(int(n[1:])) for n in g.split(".")] for g in GROUPS.split()]

    def start(after):
        for g, a in zip(groups, STARTS):
            if a == after:
                for c in g:
                    c.start()
    start(-1)
    for buf in (wqkv_r, wo_r, w1_r, w2_r, w3_r):
        buf[D:KP, :] = jnp.zeros((KP - D, buf.shape[1]), bf16)
    for name, gen in (("PQ", p_qkv(0)), ("PK", p_qkv(1)), ("PV_", p_qkv(2)), ("PWO", p_wo()),
                      ("PW1", p_plain(w1_r, w1_s, 1)), ("PW2", p_plain(w2_r, w2_s, GELU_OUT)), ("PW4", p_w4())):
        il.add((name, 0), gen)
    for c in range(NC3):
        il.add(("PW3%d" % c, 0), p_w3(c))
    for i in range(2 * NP):
        for name, gen in (("LA", g_la), ("QK", g_qk), ("PV", g_pv), ("LL", g_ll), ("SH", g_sh), ("L1", g_l1)):
            il.add((name, i), gen(i))
        n = F // 2 // NC3
        for c in range(NC3):
            il.add(("FO%d" % c, i), operands("f_op", i, "f", F // 2, F // 2, c * n, (c + 1) * n, 7))
        if i >= NP:
            il.add(("OUT", i), g_out(i))
    for name, i in order:
        if name == "DMA":
            for c in groups[i]:
                c.wait()
            il.done.add((name, i))
            start(i)
        else:
            block(name, i)
    for i in range(NP, 2 * NP):
        while ("OUT", i) in il.jobs:
            il.need(("OUT", i))
            il._step(("OUT", i))
    for j in range(NP):
        ocopy(j).wait()


@jax.jit
def pallas_interleave_layers__sliding_local_dilated__mixer_s_mlp__prompt_kernel(
        A_x, A_wqkv, A_wo, B_x, B_w1, B_w2, B_w3, B_w4):
    del B_x
    any_spec = pl.BlockSpec(memory_space=pl.ANY)
    vm = pltpu.VMEM
    dd = vm((7, K1 // 128, D // 2, 128), bf16)
    out = pl.pallas_call(
        _kernel,
        out_shape=jax.ShapeDtypeStruct((D, S), bf16),
        in_specs=[any_spec] * 7,
        out_specs=any_spec,
        scratch_shapes=[
            vm((NP, D, 2 * TT), bf16),
            vm((KP, 3 * D), bf16), vm((KP, D), bf16), vm((KP, D), bf16), vm((KP, D), bf16), vm((KP, F), bf16), vm((D, F), bf16),
            dd, dd, dd, dd, dd, dd, vm((7, K1 // 128, F // 2, 128), bf16), vm((7, F // 256, D // 2, 128), bf16),
            vm((KP // 128, 4 * D + 32, 128), f32), vm((7, 64, 128), bf16),
            vm((NP, D, 2 * TT), bf16),
            pltpu.SemaphoreType.DMA((NP,)), pltpu.SemaphoreType.DMA((7,)), pltpu.SemaphoreType.DMA((NP,)),
        ],
        compiler_params=pltpu.CompilerParams(vmem_limit_bytes=100 * 2**20),
    )(A_x.reshape(S, D).T, A_wqkv, A_wo, B_w1, B_w2, B_w3, B_w4.T)
    return out.T.reshape(1, S, D)
```
